```python
import os as _os
_os.environ.setdefault("JAX_PLATFORMS", "cpu")
import jax
import jax.numpy as jnp

def _softmax(x, axis=-1):
    return jax.nn.softmax(x, axis=axis)
def _gelu(x):
    return jax.nn.gelu(x, approximate=True)
def _silu(x):
    return jax.nn.silu(x)
def _sigmoid(x):
    return jax.nn.sigmoid(x)
def _layernorm(x, axis=-1, eps=1e-5):
    m = jnp.mean(x, axis=axis, keepdims=True)
    v = jnp.var(x, axis=axis, keepdims=True)
    return (x - m) / jnp.sqrt(v + eps)
def _scatter_add(tgt, idx, src, axis=0):
    return tgt.at[idx].add(src)
def _segment_sum(src, seg, n):
    return jax.ops.segment_sum(src, seg, n)
class _Rng:
    def __init__(self, key):
        self._k = key
    def _next(self):
        self._k, sub = jax.random.split(self._k)
        return sub
    def normal(self, shape):
        return jax.random.normal(self._next(), shape, dtype=jnp.bfloat16)
    def randint(self, lo, hi, shape):
        return jax.random.randint(self._next(), shape, lo, hi, dtype=jnp.int32)
    def uniform(self, shape, lo=0.0, hi=1.0):
        return jax.random.uniform(self._next(), shape, jnp.bfloat16, lo, hi)
    def permutation(self, n):
        return jax.random.permutation(self._next(), n)


kernel_name = 'concat_heads__linear_attn_block__sliding_local_dilated__prompt'

def setup_inputs():
    _rng = _Rng(jax.random.key(int.from_bytes(__import__("os").urandom(4), "little")))
    _w = (lambda a: (lambda t: t.astype(jnp.bfloat16) if jnp.issubdtype(t.dtype, jnp.floating) else t)(jnp.asarray(a)))
    def _A_setup():
        B, S, D = 1, 2048, 576
        return {
            "x": _w((lambda *s: _rng.normal(s) * 0.05)(B, S, D)),
            "wqkv": _w((lambda *s: _rng.normal(s) * 1.6)(D, 3 * D)),
            "wo": _w((lambda *s: _rng.normal(s) * 0.4)(D, D)),
        }
    _A_in = _A_setup()

    def _B_setup():
        B, S, D = 1, 2048, 576
        return {
            "x": _w((lambda *s: _rng.normal(s) * 0.2)(B, S, D)),
            "wqkv": _w((lambda *s: _rng.normal(s) * 0.2)(D, 3 * D)),
            "wo": _w((lambda *s: _rng.normal(s) * 0.05)(D, D)),
        }
    _B_in = _B_setup()

    return {
        "A_x": _A_in["x"],
        "A_wqkv": _A_in["wqkv"],
        "A_wo": _A_in["wo"],
        "B_x": _B_in["x"],
        "B_wqkv": _B_in["wqkv"],
        "B_wo": _B_in["wo"],
    }

def reference(A_x, A_wqkv, A_wo, B_x, B_wqkv, B_wo):
    def _A_ref(x, wqkv, wo):
        B, S, D = x.shape
        H = 32; Dh = D // H
        qkv = (lambda x, *d: x.transpose(*d))((x @ wqkv).reshape(B, S, 3, H, Dh), 2, 0, 3, 1, 4)
        q, k, v = qkv[0], qkv[1], qkv[2]
        phi = lambda t: jnp.where(t > 0, t + 1, jnp.exp(t)) + 1e-6
        pq, pk = phi(q), phi(k)
        kv = jnp.einsum("bhsd,bhse->bhde", pk, v)
        z = jnp.einsum("bhsd->bhd", pk)
        num = jnp.einsum("bhqd,bhde->bhqe", pq, kv)
        den = jnp.einsum("bhqd,bhd->bhq", pq, z)[..., None] + 1e-6
        o = num / den
        return (lambda x, *d: x.transpose(*d))(o, 0, 2, 1, 3).reshape(B, S, D) @ wo

    def _B_ref(x, wqkv, wo):
        B, S, D = x.shape
        H = 32; Dh = D // H
        W, dil = 8, 2
        qkv = (lambda x, *d: x.transpose(*d))((x @ wqkv).reshape(B, S, 3, H, Dh), 2, 0, 3, 1, 4)
        q, k, v = qkv[0], qkv[1], qkv[2]
        scale = Dh ** -0.5
        pos = jnp.arange(S)
        off = jnp.arange(W) * dil
        idx = pos[:, None] - off[None, :]
        mask = idx >= 0
        idx_c = jnp.where(mask, idx, 0).reshape(-1)
        kg = k[:, :, idx_c, :].reshape(B, H, S, W, Dh)
        vg = v[:, :, idx_c, :].reshape(B, H, S, W, Dh)
        logits = jnp.einsum("bhsd,bhswd->bhsw", q, kg) * scale
        logits = jnp.where(mask[None, None, :, :], logits, -1e9)
        attn = _softmax(logits, axis=-1)
        o = jnp.einsum("bhsw,bhswd->bhsd", attn, vg)
        return (lambda x, *d: x.transpose(*d))(o, 0, 2, 1, 3).reshape(B, S, D) @ wo

    a = _A_ref(A_x, A_wqkv, A_wo)
    b = _B_ref(B_x, B_wqkv, B_wo)
    return jnp.concatenate([a, b], axis=-1)
```

```python
import functools

import jax
import jax.numpy as jnp
import jax.experimental.pallas as pl
import jax.experimental.pallas.tpu as pltpu

S = 2048
D = 576
H = 32
DH = 18
DP = 640
NT = 16
NC = 5
W = 8
HPT = 7
PADROWS = 592

F32 = jnp.float32
BF16 = jnp.bfloat16
U32 = jnp.uint32

NT_DIMS = (((1,), (1,)), ((), ()))


def _phi(t):
    return jnp.where(t > 0, t + 1.0, jnp.exp(t)) + 1e-6


def _blk_rows(i):
    return 128 if i < 4 else 80


def _blk_valid(i):
    return 126 if i < 4 else 72


def _kernel(xa_hbm, wa_hbm, woa_hbm, xb_hbm, wb_hbm, wob_hbm, out_hbm,
            xa, xb, wa, wb, woa, wob,
            t0, t1, t2, t3, t4,
            xs0, xs1, xs2, xs3, xs4,
            os0, os1, os2, os3, os4,
            wk_a, wv_a, wq_a, wop_a, mt_a, wt_b, wot_b,
            pk, zacc, znat, zb, sq,
            k_ext, v_ext, obuf,
            isem, osem):
    tw = [t0, t1, t2, t3, t4]
    xs = [xs0, xs1, xs2, xs3, xs4]
    osl = [os0, os1, os2, os3, os4]

    in_cps = [
        pltpu.make_async_copy(wa_hbm, wa, isem.at[0]),
        pltpu.make_async_copy(xa_hbm, xa.at[pl.ds(0, D)], isem.at[1]),
        pltpu.make_async_copy(woa_hbm, woa, isem.at[2]),
        pltpu.make_async_copy(wb_hbm, wb, isem.at[3]),
        pltpu.make_async_copy(xb_hbm, xb.at[pl.ds(0, D)], isem.at[4]),
        pltpu.make_async_copy(wob_hbm, wob, isem.at[5]),
    ]
    for c in in_cps:
        c.start()
    xa[pl.ds(D, DP - D), :] = jnp.zeros((DP - D, S), BF16)
    xb[pl.ds(D, DP - D), :] = jnp.zeros((DP - D, S), BF16)

    lane = jax.lax.broadcasted_iota(jnp.int32, (8, 128), 1)

    def transpose_w(w_ref):
        for c in range(NC):
            if c < 4:
                blk = w_ref[pl.ds(128 * c, 128), :].astype(F32)
            else:
                blk = jnp.concatenate(
                    [w_ref[pl.ds(512, 64), :].astype(F32),
                     jnp.zeros((64, 3 * D), F32)], axis=0)
            tw[c][...] = blk.T

    def rows_dh(src, base, d):
        return jnp.concatenate(
            [s[pl.ds(base + d, H, stride=DH), :] for s in src], axis=1)

    def transpose_sq(dst):
        dst[...] = sq[...].T.astype(BF16)

    in_cps[0].wait()
    transpose_w(wa)
    for d in range(DH):
        wq_a[pl.ds(d * H, H), :] = rows_dh(tw, 0, d).astype(BF16)
    for i in range(NC):
        n, nv = _blk_rows(i), _blk_valid(i)
        for dst, base in ((wk_a, D), (wv_a, 2 * D)):
            v = jnp.concatenate(
                [s[pl.ds(base + 126 * i, nv), :] for s in tw], axis=1)
            v = jnp.concatenate([v, jnp.zeros((n - nv, DP), F32)], axis=0)
            dst[pl.ds(128 * i, n), :] = v.astype(BF16)
    in_cps[2].wait()
    for i in range(NC):
        n, nv = _blk_rows(i), _blk_valid(i)
        v = woa[pl.ds(126 * i, nv), :].astype(F32)
        v = jnp.concatenate([v, jnp.zeros((n - nv, D), F32)], axis=0)
        wop_a[pl.ds(128 * i, n), :] = v.astype(BF16)

    in_cps[1].wait()
    zacc[...] = jnp.zeros(zacc.shape, F32)

    def a_k_body(t, carry):
        c0 = pl.multiple_of(t * 128, 128)
        kt = jnp.dot(wk_a[...], xa[:, pl.ds(c0, 128)], preferred_element_type=F32)
        p = _phi(kt)
        pk[:, pl.ds(c0, 128)] = p.astype(BF16)
        zacc[...] += p
        return carry

    jax.lax.fori_loop(0, NT, a_k_body, 0)

    g = jax.lax.dot_general(pk[...], xa[...], NT_DIMS,
                            preferred_element_type=F32)
    z = jnp.broadcast_to(jnp.sum(zacc[...], axis=1, keepdims=True), (PADROWS, 128))
    sq[pl.ds(D, DP - D), :] = jnp.zeros((DP - D, DP), F32)
    for i in range(NC):
        n, nv = _blk_rows(i), _blk_valid(i)
        gi = g[128 * i:128 * i + n].astype(BF16)
        kv = jax.lax.dot_general(gi, wv_a[pl.ds(128 * i, n), :], NT_DIMS,
                                 preferred_element_type=F32)
        r = jax.lax.broadcasted_iota(jnp.int32, (n, n), 0)
        c = jax.lax.broadcasted_iota(jnp.int32, (n, n), 1)
        same = ((r * 3641) >> 16) == ((c * 3641) >> 16)
        kv = jnp.where(same, kv, 0.0).astype(BF16)
        mi = jnp.dot(kv, wop_a[pl.ds(128 * i, n), :], preferred_element_type=F32)
        for cc in range(NC):
            wdt = 128 if cc < 4 else 64
            tw[cc][pl.ds(126 * i, nv), pl.ds(0, wdt)] = mi[0:nv, 128 * cc:128 * cc + wdt]
        znat[pl.ds(126 * i, nv), :] = z[128 * i:128 * i + nv]
    for d in range(DH):
        zb[pl.ds(d * H, H), :] = znat[pl.ds(d, H, stride=DH), :]
        v = jnp.concatenate(
            [tw[cc][pl.ds(d, H, stride=DH), :] for cc in range(4)]
            + [tw[4][pl.ds(d, H, stride=DH), pl.ds(0, 64)], jnp.zeros((H, 64), F32)],
            axis=1)
        sq[pl.ds(d * H, H), :] = v
    transpose_sq(mt_a)

    in_cps[3].wait()
    transpose_w(wb)
    for p in range(3):
        for d in range(DH):
            wt_b[pl.ds(p * D + d * H, H), :] = rows_dh(tw, p * D, d).astype(BF16)
    in_cps[5].wait()
    for cc in range(NC):
        wdt = 128 if cc < 4 else 64
        tw[cc][pl.ds(0, D), pl.ds(0, wdt)] = wob[:, pl.ds(128 * cc, wdt)].astype(F32)
    for d in range(DH):
        v = jnp.concatenate(
            [tw[cc][pl.ds(d, H, stride=DH), :] for cc in range(4)]
            + [tw[4][pl.ds(d, H, stride=DH), pl.ds(0, 64)], jnp.zeros((H, 64), F32)],
            axis=1)
        sq[pl.ds(d * H, H), :] = v
    transpose_sq(wot_b)

    in_cps[4].wait()

    def xb_body(t, carry):
        c0 = pl.multiple_of(t * 128, 128)
        xt = xb[:, pl.ds(c0, 128)].T
        xu = pltpu.bitcast(xt, U32)
        r0 = pl.multiple_of(t * 64, 64)
        for cc in range(NC):
            xs[cc][pl.ds(r0, 64), :] = xu[:, 128 * cc:128 * cc + 128]
        return carry

    jax.lax.fori_loop(0, NT, xb_body, 0)

    def xb_tile(j):
        t = jnp.concatenate([s[pl.ds(j, 64, stride=NT), :] for s in xs], axis=1)
        return pltpu.bitcast(t, BF16)

    def b_kv_body(j, carry):
        kvt = jax.lax.dot_general(wt_b[pl.ds(D, 2 * D), :], xb_tile(j), NT_DIMS,
                                  preferred_element_type=F32)
        k_ext[j + (W - 1)] = kvt[0:D]
        v_ext[j + (W - 1)] = kvt[D:2 * D]
        return carry

    jax.lax.fori_loop(0, NT, b_kv_body, 0)

    def roll_body(i, carry):
        k_ext[i] = pltpu.roll(k_ext[i + NT], 2, 1)
        v_ext[i] = pltpu.roll(v_ext[i + NT], 2, 1)
        return carry

    jax.lax.fori_loop(0, W - 1, roll_body, 0)

    scale = float(DH) ** -0.5

    def b_att_body(j, carry):
        q = jax.lax.dot_general(wt_b[pl.ds(0, D), :], xb_tile(j), NT_DIMS,
                                preferred_element_type=F32)
        o_rows = [None] * (DH * 4)
        for gi in range(4):
            acc = [None] * W
            for d in range(DH):
                r0 = d * H + 8 * gi
                qd = q[r0:r0 + 8]
                for w in range(W):
                    term = qd * k_ext[j + (W - 1 - w), pl.ds(r0, 8), :]
                    acc[w] = term if acc[w] is None else acc[w] + term
            lg = [acc[0] * scale]
            for w in range(1, W):
                ok = jnp.logical_or(lane >= 2, j >= w)
                lg.append(jnp.where(ok, acc[w] * scale, -1e9))
            m = lg[0]
            for w in range(1, W):
                m = jnp.maximum(m, lg[w])
            e = [jnp.exp(l - m) for l in lg]
            den = e[0]
            for w in range(1, W):
                den = den + e[w]
            inv = 1.0 / den
            p = [x * inv for x in e]
            for d in range(DH):
                r0 = d * H + 8 * gi
                o = p[0] * v_ext[j + (W - 1), pl.ds(r0, 8), :]
                for w in range(1, W):
                    o = o + p[w] * v_ext[j + (W - 1 - w), pl.ds(r0, 8), :]
                o_rows[d * 4 + gi] = o
        o = jnp.concatenate(o_rows + [jnp.zeros((DP - D, 128), F32)], axis=0).astype(BF16)
        ot = jnp.dot(wot_b[pl.ds(0, D), :], o, preferred_element_type=F32)
        ot = jnp.concatenate([jnp.zeros((64, 128), F32), ot], axis=0).astype(BF16)
        ou = pltpu.bitcast(ot.T, U32)
        for cc in range(NC):
            osl[cc][pl.ds(j, 64, stride=NT), :] = ou[:, 128 * cc:128 * cc + 128]
        return carry

    jax.lax.fori_loop(0, NT, b_att_body, 0)

    lane_hi = jax.lax.broadcasted_iota(jnp.int32, (128, 128), 1) >= 64

    def out_copy(t, slot):
        r0 = pl.multiple_of(t * 128, 128)
        return pltpu.make_async_copy(obuf.at[slot], out_hbm.at[pl.ds(r0, 128), :],
                                     osem.at[slot])

    def a_out_body(t, carry):
        slot = t % 2
        c0 = pl.multiple_of(t * 128, 128)
        q = jnp.dot(wq_a[...], xa[:, pl.ds(c0, 128)], preferred_element_type=F32)
        pq = _phi(q)
        pn_rows = [None] * (DH * 4)
        for gi in range(4):
            den = None
            for d in range(DH):
                r0 = d * H + 8 * gi
                term = pq[r0:r0 + 8] * zb[pl.ds(r0, 8), :]
                den = term if den is None else den + term
            inv = 1.0 / (den + 1e-6)
            for d in range(DH):
                r0 = d * H + 8 * gi
                pn_rows[d * 4 + gi] = pq[r0:r0 + 8] * inv
        pn = jnp.concatenate(pn_rows + [jnp.zeros((DP - D, 128), F32)], axis=0).astype(BF16)
        ot = jnp.dot(mt_a[pl.ds(0, D), :], pn, preferred_element_type=F32)
        ot = jnp.concatenate([ot, jnp.zeros((64, 128), F32)], axis=0).astype(BF16).T

        @pl.when(t >= 2)
        def _():
            out_copy(t - 2, slot).wait()

        r0 = pl.multiple_of(t * 64, 64)
        obuf[slot, :, pl.ds(0, 512)] = ot[:, 0:512]
        b0 = pltpu.bitcast(osl[0][pl.ds(r0, 64), :], BF16)
        obuf[slot, :, pl.ds(512, 128)] = jnp.where(lane_hi, b0, ot[:, 512:640])
        for cc in range(1, NC):
            obuf[slot, :, pl.ds(512 + 128 * cc, 128)] = pltpu.bitcast(
                osl[cc][pl.ds(r0, 64), :], BF16)
        out_copy(t, slot).start()
        return carry

    jax.lax.fori_loop(0, NT, a_out_body, 0)
    out_copy(NT - 2, 0).wait()
    out_copy(NT - 1, 1).wait()


@jax.jit
def pallas_concat_heads__linear_attn_block__sliding_local_dilated__prompt_kernel(
    A_x: jax.Array,
    A_wqkv: jax.Array,
    A_wo: jax.Array,
    B_x: jax.Array,
    B_wqkv: jax.Array,
    B_wo: jax.Array,
):
    xa_t = A_x.reshape(S, D).T
    xb_t = B_x.reshape(S, D).T
    any_spec = pl.BlockSpec(memory_space=pl.ANY)
    scratch = (
        [pltpu.VMEM((DP, S), BF16)] * 2
        + [pltpu.VMEM((D, 3 * D), BF16)] * 2
        + [pltpu.VMEM((D, D), BF16)] * 2
        + [pltpu.VMEM((3 * D, 128), F32)] * NC
        + [pltpu.VMEM((S // 2, 128), U32)] * (2 * NC)
        + [pltpu.VMEM((PADROWS, DP), BF16)] * 2
        + [pltpu.VMEM((D, DP), BF16)]
        + [pltpu.VMEM((PADROWS, D), BF16)]
        + [pltpu.VMEM((DP, DP), BF16)]
        + [pltpu.VMEM((3 * D, DP), BF16)]
        + [pltpu.VMEM((DP, DP), BF16)]
        + [pltpu.VMEM((PADROWS, S), BF16)]
        + [pltpu.VMEM((PADROWS, 128), F32)]
        + [pltpu.VMEM((D, 128), F32)] * 2
        + [pltpu.VMEM((DP, DP), F32)]
        + [pltpu.VMEM((NT + W - 1, D, 128), F32)] * 2
        + [pltpu.VMEM((2, 128, 2 * D), BF16)]
        + [pltpu.SemaphoreType.DMA((6,)), pltpu.SemaphoreType.DMA((2,))]
    )
    out = pl.pallas_call(
        _kernel,
        out_shape=jax.ShapeDtypeStruct((S, 2 * D), BF16),
        in_specs=[any_spec] * 6,
        out_specs=any_spec,
        scratch_shapes=scratch,
        compiler_params=pltpu.CompilerParams(vmem_limit_bytes=100 * 1024 * 1024),
        name="concat_heads",
    )(xa_t, A_wqkv, A_wo, xb_t, B_wqkv, B_wo)
    return out.reshape(1, S, 2 * D)
```

```python
import functools

import jax
import jax.numpy as jnp
import jax.experimental.pallas as pl
import jax.experimental.pallas.tpu as pltpu

S = 2048
D = 576
DH = 18
DP = 640
NT = S // 128
NC = DP // 128
W = 8
NG = 4
GR = 8 * DH

F32 = jnp.float32
BF16 = jnp.bfloat16
U32 = jnp.uint32
NT_DIMS = (((1,), (1,)), ((), ()))


def _phi(t):
    return jnp.where(t > 0, t + 1.0, jnp.exp(t)) + 1e-6


def _ld(ref, r0, n):
    return pltpu.bitcast(ref.bitcast(U32)[pl.ds(r0 // 2, n // 2), :], BF16)


def _ldw(ref, r0, n):
    m = ref.shape[0] // NC
    u = ref.bitcast(U32)
    v = jnp.concatenate([u[pl.ds((c * m + r0) // 2, n // 2), :] for c in range(NC)], axis=1)
    return pltpu.bitcast(v, BF16)


def _stw(ref, r0, val):
    m = ref.shape[0] // NC
    for c in range(NC):
        ref[pl.ds(c * m + r0, val.shape[0]), :] = val[:, 128 * c:128 * c + 128]


def _interleave(main, aux, frac):
    n = max(1, int(len(main) * frac))
    done = 0
    for i, f in enumerate(main):
        f()
        upto = min(len(aux), -(-(i + 1) * len(aux) // n))
        while done < upto:
            aux[done]()
            done += 1
    for f in aux[done:]:
        f()


def _kernel(xa_hbm, wa_hbm, woa_hbm, xb_hbm, wb_hbm, wob_hbm, out_hbm,
            xa, xb, waq, wak, wav, wb, woa, wob,
            t0, t1, t2, t3, t4, u0, u1, u2, u3, u4, s0, s1, s2, s3, s4,
            xs0, xs1, xs2, xs3, xs4, os0, os1, os2, os3, os4, ob0, ob1, ob2, ob3, ob4,
            wk_a, wv_a, wq_a, wo_a, mt_a, wt_b, wot_b,
            pk, gbuf, zacc, zb, k_ext, v_ext, q_0, q_1, o_0, o_1, pn,
            isem, xasem, osem):
    P = functools.partial
    tw = [t0, t1, t2, t3, t4]
    tu = [u0, u1, u2, u3, u4]
    sq = [s0, s1, s2, s3, s4]
    xs = [xs0, xs1, xs2, xs3, xs4]
    osl = [os0, os1, os2, os3, os4]
    obuf = [ob0, ob1, ob2, ob3, ob4]

    def x_copy(src, dst, t, sem):
        return pltpu.make_async_copy(src.at[:, pl.ds(128 * t, 128)], dst.at[pl.ds(DP * t, D), :], sem)

    cp_wak = pltpu.make_async_copy(wa_hbm.at[:, pl.ds(512, DP)], wak, isem.at[0])
    xg = (0, 2, 7, NT)
    cp_xa = [[x_copy(xa_hbm, xa, t, xasem.at[i]) for t in range(xg[i], xg[i + 1])] for i in range(3)]
    cp_b1 = [pltpu.make_async_copy(wb_hbm, wb, isem.at[1]),
             pltpu.make_async_copy(xb_hbm, xb.at[pl.ds(0, D), :], isem.at[2])]
    cp_b2 = [pltpu.make_async_copy(wa_hbm.at[:, pl.ds(0, DP)], waq, isem.at[3]),
             pltpu.make_async_copy(wa_hbm.at[:, pl.ds(2 * D, D)], wav, isem.at[4]),
             pltpu.make_async_copy(woa_hbm, woa, isem.at[5]),
             pltpu.make_async_copy(wob_hbm, wob, isem.at[6])]

    def start(cps):
        for c in cps:
            c.start()

    def wait(cps):
        for c in cps:
            c.wait()

    cp_wak.start()
    start(cp_xa[0])
    for t in range(NT):
        for r in (xa, pn):
            r[pl.ds(DP * t + D, DP - D), :] = jnp.zeros((DP - D, 128), BF16)
    xb[pl.ds(D, DP - D), :] = jnp.zeros((DP - D, S), BF16)
    for r in (o_0, o_1):
        r[pl.ds(D, DP - D), :] = jnp.zeros((DP - D, 128), BF16)
    for r in sq:
        r[pl.ds(D, DP - D), :] = jnp.zeros((DP - D, 128), F32)
    zacc[...] = jnp.zeros(zacc.shape, F32)
    lane = jax.lax.broadcasted_iota(jnp.int32, (8, 128), 1)

    def x_tile(ref, t):
        return _ld(ref, DP * t, DP)

    def w_slab(w_ref, c0, ncols, dst, row0, c):
        if c < 4:
            blk = w_ref[pl.ds(128 * c, 128), pl.ds(c0, ncols)].astype(F32)
        else:
            blk = jnp.concatenate(
                [w_ref[pl.ds(512, 64), pl.ds(c0, ncols)].astype(F32), jnp.zeros((64, ncols), F32)], axis=0)
        dst[c][pl.ds(row0, ncols), :] = blk.T

    def wo_slab(w_ref, dst, c):
        if c < 4:
            v = w_ref[:, pl.ds(128 * c, 128)].astype(F32)
        else:
            v = jnp.concatenate([w_ref[:, pl.ds(512, 64)].astype(F32), jnp.zeros((D, 64), F32)], axis=1)
        dst[c][pl.ds(0, D), :] = v

    def rows_f(src, base):
        return jnp.concatenate(
            [jnp.concatenate([s[pl.ds(base + d, 8, stride=DH), :] for s in src], axis=1)
             for d in range(DH)], axis=0)

    def prep_g(src, base, dst, r0, g):
        _stw(dst, r0 + GR * g, rows_f(src, base + GR * g).astype(BF16))

    def sq_rows(src, g):
        v = rows_f(src, GR * g)
        for cc in range(NC):
            sq[cc][pl.ds(GR * g, GR), :] = v[:, 128 * cc:128 * cc + 128]

    def sq_t(dst, c):
        v = jnp.concatenate([sq[cc][pl.ds(128 * c, 128), :] for cc in range(NC)], axis=1)
        dst[pl.ds(c * D, D), :] = v.T[0:D].astype(BF16)

    def prep_k(g):
        c0 = (64 + GR * g) // 128 * 128
        for c in range(NC):
            w_slab(wak, c0, 256, tw, 256 * g, c)
        _stw(wk_a, GR * g, rows_f(tw, 256 * g + 64 + GR * g - c0).astype(BF16))

    def a_k(t, g):
        p = _phi(jnp.dot(_ldw(wk_a, GR * g, GR), x_tile(xa, t), preferred_element_type=F32))
        pk[pl.ds(D * t + GR * g, GR), :] = p.astype(BF16)
        zacc[pl.ds(GR * g, GR), :] += p

    cp_wak.wait()
    start(cp_xa[1] + cp_xa[2])
    prep_k(0)
    prep_k(1)
    wait(cp_xa[0])
    a_k(0, 0)
    prep_k(2)
    a_k(1, 0)
    a_k(0, 1)
    prep_k(3)
    a_k(1, 1)
    for t in range(2):
        for g in (2, 3):
            a_k(t, g)

    for t in range(2, NT):
        if t == xg[1]:
            wait(cp_xa[1])
            start(cp_b1)
        if t == xg[2]:
            wait(cp_xa[2])
        if t == 9:
            start(cp_b2)
        for g in range(NG):
            a_k(t, g)

    def g_mm(g, c):
        pk_g = jnp.concatenate([_ld(pk, D * t + GR * g, GR) for t in range(NT)], axis=1)
        xa_c = jnp.concatenate([_ld(xa, DP * t + 128 * c, 128) for t in range(NT)], axis=1)
        gg = jax.lax.dot_general(pk_g, xa_c, NT_DIMS, preferred_element_type=F32)
        gbuf[pl.ds(c * D + GR * g, GR), :] = gg.astype(BF16)

    def xb_rows(t):
        xu = pltpu.bitcast(xb[:, pl.ds(128 * t, 128)].T, U32)
        for cc in range(NC):
            for a in range(4):
                xs[cc][pl.ds(4 * t + a, 16, stride=64), :] = xu[16 * a:16 * a + 16, 128 * cc:128 * cc + 128]

    def xb_tile(j):
        return pltpu.bitcast(jnp.concatenate([s[pl.ds(64 * j, 64), :] for s in xs], axis=1), BF16)

    g_tasks = [P(g_mm, g, c) for c in range(NC) for g in range(NG)]
    aux = [P(xb_rows, t) for t in range(NT)]
    aux += [P(w_slab, wb, 512, 3 * D - 512, tu, 512, c) for c in range(NC)]
    aux += [P(prep_g, tu, p * D, wt_b, p * D, g) for p in (1, 2) for g in range(NG)]
    for f in g_tasks[:5]:
        f()
    wait(cp_b1)
    _interleave(g_tasks[5:], aux, 0.9)

    def m_chain(g):
        kv = jax.lax.dot_general(_ldw(gbuf, GR * g, GR), _ldw(wv_a, GR * g, GR), NT_DIMS,
                                 preferred_element_type=F32)
        r = jax.lax.broadcasted_iota(jnp.int32, (GR, GR), 0)
        c = jax.lax.broadcasted_iota(jnp.int32, (GR, GR), 1)
        kv = jnp.where((r & 7) == (c & 7), kv, 0.0).astype(BF16)
        m = jnp.dot(kv, _ldw(wo_a, GR * g, GR), preferred_element_type=F32)
        for cc in range(NC):
            sq[cc][pl.ds(GR * g, GR), :] = m[:, 128 * cc:128 * cc + 128]

    def z_bcast():
        zb[...] = jnp.broadcast_to(jnp.sum(zacc[...], axis=1, keepdims=True), (D, 128))

    def b_kv(j, p, g):
        ext = k_ext if p == 1 else v_ext
        r = jax.lax.dot_general(_ldw(wt_b, p * D + GR * g, GR), xb_tile(j), NT_DIMS,
                                preferred_element_type=F32)
        ext[j + (W - 1), pl.ds(GR * g, GR), :] = r
        if j >= NT - (W - 1):
            ext[j - (NT - (W - 1)), pl.ds(GR * g, GR), :] = pltpu.roll(r, 2, 1)

    wait(cp_b2)
    kv_tasks = [P(b_kv, j, p, g) for j in range(NT) for p in (1, 2) for g in range(NG)]
    aux = [P(w_slab, wav, 0, D, tw, 0, c) for c in range(NC)]
    aux += [P(prep_g, tw, 0, wv_a, 0, g) for g in range(NG)]
    aux += [P(wo_slab, woa, tw, c) for c in range(NC)]
    aux += [P(prep_g, tw, 0, wo_a, 0, g) for g in range(NG)]
    aux += [P(m_chain, g) for g in range(NG)]
    aux += [P(sq_t, mt_a, c) for c in range(NC)]
    aux += [P(w_slab, wb, 0, 512, tu, 0, c) for c in range(NC)]
    aux += [P(prep_g, tu, 0, wt_b, 0, g) for g in range(NG)]
    aux += [P(w_slab, waq, 0, DP, tw, 0, c) for c in range(NC)]
    aux += [P(prep_g, tw, 0, wq_a, 0, g) for g in range(NG)]
    aux += [z_bcast]
    aux += [P(wo_slab, wob, tu, c) for c in range(NC)]
    aux += [P(sq_rows, tu, g) for g in range(NG)]
    aux += [P(sq_t, wot_b, c) for c in range(NC)]
    _interleave(kv_tasks, aux, 0.9)

    scale = float(DH) ** -0.5

    def b_q(j, g, q_ref):
        q_ref[...] = jax.lax.dot_general(_ldw(wt_b, GR * g, GR), xb_tile(j), NT_DIMS,
                                         preferred_element_type=F32)

    def b_att(j, g, q_ref, o_ref):
        acc = [None] * W
        for d in range(DH):
            r0 = GR * g + 8 * d
            qd = q_ref[pl.ds(8 * d, 8), :]
            for w in range(W):
                term = qd * k_ext[j + (W - 1 - w), pl.ds(r0, 8), :]
                acc[w] = term if acc[w] is None else acc[w] + term
        lg = [acc[w] * scale if j >= w else jnp.where(lane >= 2, acc[w] * scale, -1e9) for w in range(W)]
        m = lg[0]
        for w in range(1, W):
            m = jnp.maximum(m, lg[w])
        e = [jnp.exp(x - m) for x in lg]
        den = e[0]
        for w in range(1, W):
            den = den + e[w]
        inv = 1.0 / den
        p = [x * inv for x in e]
        outs = []
        for d in range(DH):
            r0 = GR * g + 8 * d
            o = p[0] * v_ext[j + (W - 1), pl.ds(r0, 8), :]
            for w in range(1, W):
                o = o + p[w] * v_ext[j + (W - 1 - w), pl.ds(r0, 8), :]
            outs.append(o)
        o_ref[pl.ds(GR * g, GR), :] = jnp.concatenate(outs, axis=0).astype(BF16)

    def b_out(j, c, o_ref):
        if c == 1:
            ot = jnp.dot(_ldw(wot_b, 0, 192), _ld(o_ref, 0, DP), preferred_element_type=F32)
            o0 = jnp.concatenate([jnp.zeros((64, 128), F32), ot[0:64]], axis=0)
            osl[0][pl.ds(j, 64, stride=NT), :] = pltpu.bitcast(o0.astype(BF16).T, U32)
            ot = ot[64:192]
        else:
            ot = jnp.dot(_ldw(wot_b, 128 * c - 64, 128), _ld(o_ref, 0, DP), preferred_element_type=F32)
        osl[c][pl.ds(j, 64, stride=NT), :] = pltpu.bitcast(ot.astype(BF16).T, U32)

    def a_q(t, g):
        pq = _phi(jnp.dot(_ldw(wq_a, GR * g, GR), x_tile(xa, t), preferred_element_type=F32))
        prod = pq * zb[pl.ds(GR * g, GR), :]
        den = prod[0:8]
        for d in range(1, DH):
            den = den + prod[8 * d:8 * d + 8]
        inv = 1.0 / (den + 1e-6)
        pn[pl.ds(DP * t + GR * g, GR), :] = (pq * jnp.concatenate([inv] * DH, axis=0)).astype(BF16)

    steps = [(j, g) for j in range(NT) for g in range(NG)]
    qr = (q_0, q_1)
    orf = (o_0, o_1)
    out_chunks = ((1,), (2,), (3,), (4,))
    b_q(0, 0, qr[0])
    for i, (j, g) in enumerate(steps):
        if j > 0:
            for c in out_chunks[g]:
                b_out(j - 1, c, orf[(j - 1) % 2])
        a_q(j, g)
        if i + 1 < len(steps):
            b_q(*steps[i + 1], qr[(i + 1) % 2])
        b_att(j, g, qr[i % 2], orf[j % 2])
    for c in range(1, NC):
        b_out(NT - 1, c, orf[(NT - 1) % 2])

    lane_hi = jax.lax.broadcasted_iota(jnp.int32, (64, 128), 1) >= 64
    b_cps = [pltpu.make_async_copy(osl[c].bitcast(BF16).at[pl.ds(0, S), :],
                                   out_hbm.at[:, pl.ds(512 + 128 * c, 128)], osem.at[1])
             for c in range(1, NC)]
    start(b_cps)

    def out_copy(t, c):
        src = obuf[c] if c < 4 else obuf[c].bitcast(BF16)
        return pltpu.make_async_copy(src.at[pl.ds(128 * t, 128), :],
                                     out_hbm.at[pl.ds(128 * t, 128), pl.ds(128 * c, 128)], osem.at[0])

    def a_out(t, c):
        pt = _ld(pn, DP * t, DP)
        if c < 3:
            ot = jnp.dot(_ldw(mt_a, 128 * c, 128), pt, preferred_element_type=F32)
        else:
            ot = jnp.dot(_ldw(mt_a, 384, 192), pt, preferred_element_type=F32)
            o4 = jnp.concatenate([ot[128:192], jnp.zeros((64, 128), F32)], axis=0)
            obuf[4][pl.ds(64 * t, 64), :] = jnp.where(
                lane_hi, osl[0][pl.ds(64 * t, 64), :], pltpu.bitcast(o4.astype(BF16).T, U32))
            out_copy(t, 4).start()
            ot = ot[0:128]
        obuf[c][pl.ds(128 * t, 128), :] = ot.astype(BF16).T
        out_copy(t, c).start()

    for t in range(NT):
        for c in range(4):
            a_out(t, c)
    wait(b_cps)
    wait([out_copy(t, c) for t in range(NT) for c in range(NC)])


@jax.jit
def pallas_concat_heads__linear_attn_block__sliding_local_dilated__prompt_kernel(
    A_x: jax.Array,
    A_wqkv: jax.Array,
    A_wo: jax.Array,
    B_x: jax.Array,
    B_wqkv: jax.Array,
    B_wo: jax.Array,
):
    xa_t = A_x.reshape(S, D).T
    xb_t = B_x.reshape(S, D).T
    V = pltpu.VMEM
    scratch = (
        [V((NT * DP, 128), BF16), V((DP, S), BF16)]
        + [V((D, DP), BF16)] * 2 + [V((D, D), BF16)]
        + [V((D, 3 * D), BF16)]
        + [V((D, D), BF16)] * 2
        + [V((1048, 128), F32)] * NC
        + [V((3 * D + 24, 128), F32)] * NC
        + [V((DP, 128), F32)] * NC
        + [V((S // 2 + 64, 128), U32)] * (2 * NC)
        + [V((S, 128), BF16)] * 4 + [V((S // 2, 128), U32)]
        + [V((NC * D, 128), BF16)] * 5
        + [V((NC * 3 * D, 128), BF16)]
        + [V((NC * D, 128), BF16)]
        + [V((NT * D, 128), BF16)]
        + [V((NC * D, 128), BF16)]
        + [V((D, 128), F32)] * 2
        + [V((NT + W - 1, D, 128), F32)] * 2
        + [V((GR, 128), F32)] * 2
        + [V((DP, 128), BF16)] * 2
        + [V((NT * DP, 128), BF16)]
        + [pltpu.SemaphoreType.DMA((7,)), pltpu.SemaphoreType.DMA((3,)), pltpu.SemaphoreType.DMA((2,))]
    )
    any_spec = pl.BlockSpec(memory_space=pl.ANY)
    out = pl.pallas_call(
        _kernel,
        out_shape=jax.ShapeDtypeStruct((S, 2 * D), BF16),
        in_specs=[any_spec] * 6,
        out_specs=any_spec,
        scratch_shapes=scratch,
        compiler_params=pltpu.CompilerParams(
            vmem_limit_bytes=100 * 1024 * 1024,
            flags={"XLA_TPU_EVENLY_DISTRIBUTE_CRITICAL_NODES": True}),
        name="concat_heads",
    )(xa_t, A_wqkv, A_wo, xb_t, B_wqkv, B_wo)
    return out.reshape(1, S, 2 * D)
```
